```python
import jax
import jax.numpy as jnp

def _softmax(x, axis=-1):
    return jax.nn.softmax(x, axis=axis)
def _gelu(x):
    return jax.nn.gelu(x, approximate=True)
def _silu(x):
    return jax.nn.silu(x)
def _sigmoid(x):
    return jax.nn.sigmoid(x)
def _layernorm(x, axis=-1, eps=1e-5):
    m = jnp.mean(x, axis=axis, keepdims=True)
    v = jnp.var(x, axis=axis, keepdims=True)
    return (x - m) / jnp.sqrt(v + eps)
def _scatter_add(tgt, idx, src, axis=0):
    return tgt.at[idx].add(src)
def _segment_sum(src, seg, n):
    return jax.ops.segment_sum(src, seg, n)
class _Rng:
    def __init__(self, key):
        self._k = key
    def _next(self):
        self._k, sub = jax.random.split(self._k)
        return sub
    def normal(self, shape):
        return jax.random.normal(self._next(), shape, dtype=jnp.bfloat16)
    def randint(self, lo, hi, shape):
        return jax.random.randint(self._next(), shape, lo, hi, dtype=jnp.int32)
    def uniform(self, shape, lo=0.0, hi=1.0):
        return jax.random.uniform(self._next(), shape, jnp.bfloat16, lo, hi)
    def permutation(self, n):
        return jax.random.permutation(self._next(), n)


kernel_name = 'concat_heads__gqa_block_cached__gqa_block_cached__near_ridge'

def setup_inputs():
    _rng = _Rng(jax.random.key(int.from_bytes(__import__("os").urandom(4), "little")))
    _w = (lambda a: (lambda t: t.astype(jnp.bfloat16) if jnp.issubdtype(t.dtype, jnp.floating) else t)(jnp.asarray(a)))
    def _A_setup():
        B, Sq, D = 8, 256, 640
        Hq, Hkv, Sk, Dh = 32, 32, 1024, 192
        assert Hq % Hkv == 0, (Hq, Hkv)
        return {
            "x": _w((lambda *s: _rng.normal(s) * 0.05)(B, Sq, D)),
            "k_cache": _w((lambda *s: _rng.normal(s) * 0.05)(B, Hkv, Sk, Dh)),
            "v_cache": _w((lambda *s: _rng.normal(s) * 0.05)(B, Hkv, Sk, Dh)),
            "wq": _w((lambda *s: _rng.normal(s) * 0.05)(D, Hq * Dh) * (D ** -0.5)),
            "wo": _w((lambda *s: _rng.normal(s) * 0.05)(Hq * Dh, D) * ((Hq * Dh) ** -0.5)),
        }
    _A_in = _A_setup()

    def _B_setup():
        B, Sq, D = 8, 256, 640
        Hq, Hkv, Sk, Dh = 32, 32, 1024, 192
        assert Hq % Hkv == 0, (Hq, Hkv)
        return {
            "x": _w((lambda *s: _rng.normal(s) * 0.05)(B, Sq, D)),
            "k_cache": _w((lambda *s: _rng.normal(s) * 0.05)(B, Hkv, Sk, Dh)),
            "v_cache": _w((lambda *s: _rng.normal(s) * 0.05)(B, Hkv, Sk, Dh)),
            "wq": _w((lambda *s: _rng.normal(s) * 0.05)(D, Hq * Dh) * (D ** -0.5)),
            "wo": _w((lambda *s: _rng.normal(s) * 0.05)(Hq * Dh, D) * ((Hq * Dh) ** -0.5)),
        }
    _B_in = _B_setup()

    return {
        "A_x": _A_in["x"],
        "A_k_cache": _A_in["k_cache"],
        "A_v_cache": _A_in["v_cache"],
        "A_wq": _A_in["wq"],
        "A_wo": _A_in["wo"],
        "B_x": _B_in["x"],
        "B_k_cache": _B_in["k_cache"],
        "B_v_cache": _B_in["v_cache"],
        "B_wq": _B_in["wq"],
        "B_wo": _B_in["wo"],
    }

def reference(A_x, A_k_cache, A_v_cache, A_wq, A_wo, B_x, B_k_cache, B_v_cache, B_wq, B_wo):
    def _A_ref(x, k_cache, v_cache, wq, wo):
        B, Sq, D = x.shape
        Hq, Dh = 32, 192
        Hkv = k_cache.shape[1]
        rep = Hq // Hkv
        q = (lambda x, *d: x.transpose(*d))((x @ wq).reshape(B, Sq, Hq, Dh), 0, 2, 1, 3)
        k = jnp.repeat(k_cache, rep, axis=1)
        v = jnp.repeat(v_cache, rep, axis=1)
        scores = jnp.einsum("bhqd,bhkd->bhqk", q, k) * (Dh ** -0.5)
        p = _softmax(scores, axis=-1)
        o = jnp.einsum("bhqk,bhkd->bhqd", p, v)
        return (lambda x, *d: x.transpose(*d))(o, 0, 2, 1, 3).reshape(B, Sq, Hq * Dh) @ wo

    def _B_ref(x, k_cache, v_cache, wq, wo):
        B, Sq, D = x.shape
        Hq, Dh = 32, 192
        Hkv = k_cache.shape[1]
        rep = Hq // Hkv
        q = (lambda x, *d: x.transpose(*d))((x @ wq).reshape(B, Sq, Hq, Dh), 0, 2, 1, 3)
        k = jnp.repeat(k_cache, rep, axis=1)
        v = jnp.repeat(v_cache, rep, axis=1)
        scores = jnp.einsum("bhqd,bhkd->bhqk", q, k) * (Dh ** -0.5)
        p = _softmax(scores, axis=-1)
        o = jnp.einsum("bhqk,bhkd->bhqd", p, v)
        return (lambda x, *d: x.transpose(*d))(o, 0, 2, 1, 3).reshape(B, Sq, Hq * Dh) @ wo

    a = _A_ref(A_x, A_k_cache, A_v_cache, A_wq, A_wo)
    b = _B_ref(B_x, B_k_cache, B_v_cache, B_wq, B_wo)
    return jnp.concatenate([a, b], axis=-1)
```

```python
import functools
import math
import jax
import jax.numpy as jnp
import jax.experimental.pallas as pl
import jax.experimental.pallas.tpu as pltpu

B, SQ, D, H, SK, DH = 8, 256, 640, 32, 1024, 192
LOG2E = 1.4426950408889634


def make(hb=4, vmem=100, peel=1):
    HG = H // hb
    qscale = (DH ** -0.5) * LOG2E
    HD = hb * DH

    def kern(xa_h, ka_h, va_h, wqa_h, woa_h, xb_h, kb_h, vb_h, wqb_h, wob_h, o_h,
             acc_ref, x_buf, k_buf, v_buf, wq_buf, wo_buf, o_buf, s_step, s_w, s_o):
        xs_h = (xa_h, xb_h)
        ks_h = (ka_h, kb_h)
        vs_h = (va_h, vb_h)
        wqs_h = (wqa_h, wqb_h)
        wos_h = (woa_h, wob_h)

        def x_cp(s, b, slot):
            return pltpu.make_async_copy(xs_h[s].at[b], x_buf.at[slot, s], s_step.at[slot, s])

        def k_cp(s, g, b, slot):
            return pltpu.make_async_copy(ks_h[s].at[b, pl.ds(pl.multiple_of(g * HD, HD), HD)],
                                         k_buf.at[slot, s], s_step.at[slot, 2 + s])

        def v_cp(s, g, b, slot):
            return pltpu.make_async_copy(vs_h[s].at[b, pl.ds(pl.multiple_of(g * HD, HD), HD)],
                                         v_buf.at[slot, s], s_step.at[slot, 4 + s])

        def wq_cp(s, g, slot):
            return pltpu.make_async_copy(wqs_h[s].at[:, pl.ds(pl.multiple_of(g * HD, HD), HD)],
                                         wq_buf.at[slot, s], s_w.at[slot, s])

        def wo_cp(s, g, slot):
            return pltpu.make_async_copy(wos_h[s].at[pl.ds(pl.multiple_of(g * HD, HD), HD), :],
                                         wo_buf.at[slot, s], s_w.at[slot, 2 + s])

        def o_cp(b):
            return pltpu.make_async_copy(o_buf.at[b], o_h.at[b], s_o.at[b])

        def start_step(g, b, slot):
            x_cp(0, b, slot).start()
            x_cp(1, b, slot).start()
            k_cp(0, g, b, slot).start()
            k_cp(1, g, b, slot).start()
            v_cp(0, g, b, slot).start()
            v_cp(1, g, b, slot).start()

        x_cp(0, 0, 0).start()
        wq_cp(0, 0, 0).start()
        x_cp(1, 0, 0).start()
        wq_cp(1, 0, 0).start()
        if not peel:
            k_cp(0, 0, 0, 0).start()
            k_cp(1, 0, 0, 0).start()
        for bb in range(B):
            acc_ref[bb] = jnp.zeros((SQ, 2 * D), jnp.float32)
        if peel:
            wq_cp(0, 0, 0).wait()
            wq_cp(1, 0, 0).wait()
            k_cp(0, 0, 0, 0).start()
            k_cp(1, 0, 0, 0).start()
        v_cp(0, 0, 0, 0).start()
        v_cp(1, 0, 0, 0).start()
        wo_cp(0, 0, 0).start()
        wo_cp(1, 0, 0).start()

        lane = jax.lax.broadcasted_iota(jnp.int32, (SQ, 128), 1)

        def step(g, b, first):
            ws = g % 2
            if True:
                slot = b % 2
                i1 = g * B + b + 1
                last = i1 >= HG * B
                g1 = jnp.where(last, g, i1 // B)
                b1 = jnp.where(last, b, i1 % B)
                if not first:
                    start_step(g1, b1, 1 - slot)

                tasks = []
                if True:
                    for j in range(hb // 2):
                        for s in range(2):
                            tasks.append((s, 2 * j))
                            tasks.append((s, 2 * j + 1))
                n = len(tasks)
                qp, S, P, RL, OT, ON = {}, {}, {}, {}, {}, {}
                waited = set()

                def need(name, s):
                    if (name, s) in waited:
                        return
                    waited.add((name, s))
                    if name == 'x':
                        x_cp(s, b, slot).wait()
                    elif name == 'k':
                        k_cp(s, g, b, slot).wait()
                    elif name == 'v':
                        v_cp(s, g, b, slot).wait()
                        if s == 1 and first:
                            start_step(g1, b1, 1 - slot)
                    elif name == 'wo' and s == 0:
                        wo_cp(0, g, ws).wait()
                        wo_cp(1, g, ws).wait()

                if not first:
                    for nm in 'xkv':
                        for s in range(2):
                            need(nm, s)

                def qproj(s):
                    need('x', s)
                    q = jnp.dot(x_buf[slot, s], wq_buf[ws, s], preferred_element_type=jnp.float32) * qscale
                    q = q.astype(jnp.bfloat16)
                    for j in range(hb // 2):
                        q0 = q[:, 384 * j:384 * j + 128]
                        q1 = q[:, 384 * j + 128:384 * j + 256]
                        q2 = q[:, 384 * j + 256:384 * j + 384]
                        zero = jnp.zeros_like(q1)
                        qp[(s, 2 * j)] = jnp.concatenate([q0, jnp.where(lane < 64, q1, zero)], axis=1)
                        qp[(s, 2 * j + 1)] = jnp.concatenate([jnp.where(lane >= 64, q1, zero), q2], axis=1)

                def qk(t):
                    s, h = tasks[t]
                    need('k', s)
                    r0 = 384 * (h // 2) + 128 * (h % 2)
                    S[t] = jnp.dot(qp.pop((s, h)), k_buf[slot, s, r0:r0 + 256, :],
                                   preferred_element_type=jnp.float32)

                def sm(t):
                    s_ = S.pop(t)
                    m = jnp.max(s_, axis=1, keepdims=True)
                    p = jnp.exp2(s_ - m)
                    l = jnp.sum(p, axis=1, keepdims=True)
                    P[t] = p.astype(jnp.bfloat16)
                    RL[t] = 1.0 / l

                def pv(t):
                    s, h = tasks[t]
                    need('v', s)
                    OT[t] = jax.lax.dot_general(v_buf[slot, s, h * DH:(h + 1) * DH, :], P.pop(t),
                                                (((1,), (1,)), ((), ())),
                                                preferred_element_type=jnp.float32)

                def tr(t):
                    o = jnp.concatenate([OT.pop(t - 1), OT.pop(t)], axis=0).T
                    lane3 = jax.lax.broadcasted_iota(jnp.int32, (SQ, 384), 1)
                    o = o * jnp.where(lane3 < 192, RL.pop(t - 1), RL.pop(t))
                    ON[t] = o.astype(jnp.bfloat16)

                def op_all(s):
                    ts = [t for t in range(1, n, 2) if tasks[t][0] == s]
                    if first:
                        need('wo', s)
                    o = jnp.concatenate([ON.pop(t) for t in ts], axis=1)
                    r = jnp.dot(o, wo_buf[ws, s], preferred_element_type=jnp.float32)
                    acc_ref[b, :, s * D:(s + 1) * D] += r

                qb, oa = -1, n
                qproj(0)
                if qb < 0:
                    qproj(1)
                qk(0)
                for u in range(n + 1):
                    if u == qb:
                        qproj(1)
                    if u + 1 < n:
                        qk(u + 1)
                    if u < n:
                        sm(u)
                    if u == oa:
                        op_all(0)
                    if 0 <= u - 1 < n:
                        pv(u - 1)
                        if (u - 1) % 2 == 1:
                            tr(u - 1)
                if oa > n:
                    op_all(0)
                op_all(1)

                @pl.when(g == HG - 1)
                def _():
                    o_buf[b] = acc_ref[b].astype(jnp.bfloat16)
                    o_cp(b).start()


        def g_body(g, _):
            ws = g % 2

            @pl.when(g >= peel)
            def _():
                wq_cp(0, g, ws).wait()
                wq_cp(1, g, ws).wait()
                wo_cp(0, g, ws).wait()
                wo_cp(1, g, ws).wait()

            @pl.when(g + 1 < HG)
            def _():
                wq_cp(0, g + 1, 1 - ws).start()
                wq_cp(1, g + 1, 1 - ws).start()
                wo_cp(0, g + 1, 1 - ws).start()
                wo_cp(1, g + 1, 1 - ws).start()

            def b_body(b, _):
                step(g, b, False)
                return 0
            jax.lax.fori_loop(jnp.where(g == 0, peel, 0), B, b_body, 0)
            return 0

        if peel:
            step(0, 0, True)
        jax.lax.fori_loop(0, HG, g_body, 0)
        x_cp(0, 0, 0).wait()
        x_cp(1, 0, 0).wait()
        k_cp(0, 0, 0, 0).wait()
        k_cp(1, 0, 0, 0).wait()
        v_cp(0, 0, 0, 0).wait()
        v_cp(1, 0, 0, 0).wait()
        for bb in range(B):
            o_cp(bb).wait()

    def fn(A_x, A_k, A_v, A_wq, A_wo, B_x, B_k, B_v, B_wq, B_wo):
        t = lambda a: jnp.swapaxes(a, 2, 3).reshape(B, H * DH, SK)
        anys = pl.BlockSpec(memory_space=pl.ANY)
        return pl.pallas_call(
            kern,
            in_specs=[anys] * 10,
            out_specs=anys,
            out_shape=jax.ShapeDtypeStruct((B, SQ, 2 * D), jnp.bfloat16),
            scratch_shapes=[
                pltpu.VMEM((B, SQ, 2 * D), jnp.float32),
                pltpu.VMEM((2, 2, SQ, D), jnp.bfloat16),
                pltpu.VMEM((2, 2, HD, SK), jnp.bfloat16),
                pltpu.VMEM((2, 2, HD, SK), jnp.bfloat16),
                pltpu.VMEM((2, 2, D, HD), jnp.bfloat16),
                pltpu.VMEM((2, 2, HD, D), jnp.bfloat16),
                pltpu.VMEM((B, SQ, 2 * D), jnp.bfloat16),
                pltpu.SemaphoreType.DMA((2, 6)),
                pltpu.SemaphoreType.DMA((2, 4)),
                pltpu.SemaphoreType.DMA((B,)),
            ],
            compiler_params=pltpu.CompilerParams(
                vmem_limit_bytes=vmem * 1024 * 1024),
        )(A_x, t(A_k), t(A_v), A_wq, A_wo, B_x, t(B_k), t(B_v), B_wq, B_wo)
    return fn


@jax.jit
def pallas_concat_heads__gqa_block_cached__gqa_block_cached__near_ridge_kernel(
        A_x, A_k_cache, A_v_cache, A_wq, A_wo, B_x, B_k_cache, B_v_cache, B_wq, B_wo):
    return make()(A_x, A_k_cache, A_v_cache, A_wq, A_wo, B_x, B_k_cache, B_v_cache, B_wq, B_wo)
```

```python
import functools
import math
import jax
import jax.numpy as jnp
import jax.experimental.pallas as pl
import jax.experimental.pallas.tpu as pltpu

B, SQ, D, H, SK, DH = 8, 256, 640, 32, 1024, 192
LOG2E = 1.4426950408889634


def make(hb=4, vmem=100, peel=1, spos=1, oa=8, nb=True):
    HG = H // hb
    qscale = (DH ** -0.5) * LOG2E
    HD = hb * DH

    def kern(xa_h, ka_h, va_h, wqa_h, woa_h, xb_h, kb_h, vb_h, wqb_h, wob_h, o_h,
             acc_ref, x_buf, k_buf, v_buf, wq_buf, wo_buf, o_buf, s_step, s_w, s_o):
        xs_h = (xa_h, xb_h)
        ks_h = (ka_h, kb_h)
        vs_h = (va_h, vb_h)
        wqs_h = (wqa_h, wqb_h)
        wos_h = (woa_h, wob_h)

        def x_cp(s, b, slot):
            return pltpu.make_async_copy(xs_h[s].at[b], x_buf.at[slot, s], s_step.at[slot, s])

        def k_cp(s, g, b, slot):
            return pltpu.make_async_copy(ks_h[s].at[b, pl.ds(pl.multiple_of(g * HD, HD), HD)],
                                         k_buf.at[slot, s], s_step.at[slot, 2 + s])

        def v_cp(s, g, b, slot):
            return pltpu.make_async_copy(vs_h[s].at[b, pl.ds(pl.multiple_of(g * HD, HD), HD)],
                                         v_buf.at[slot, s], s_step.at[slot, 4 + s])

        def wq_cp(s, g, slot):
            return pltpu.make_async_copy(wqs_h[s].at[:, pl.ds(pl.multiple_of(g * HD, HD), HD)],
                                         wq_buf.at[slot, s], s_w.at[slot, s])

        def wo_cp(s, g, slot):
            return pltpu.make_async_copy(wos_h[s].at[pl.ds(pl.multiple_of(g * HD, HD), HD), :],
                                         wo_buf.at[slot, s], s_w.at[slot, 2 + s])

        def o_cp(b):
            return pltpu.make_async_copy(o_buf.at[b], o_h.at[b], s_o.at[b])

        def start_step(g, b, slot):
            x_cp(0, b, slot).start()
            x_cp(1, b, slot).start()
            k_cp(0, g, b, slot).start()
            k_cp(1, g, b, slot).start()
            v_cp(0, g, b, slot).start()
            v_cp(1, g, b, slot).start()

        x_cp(0, 0, 0).start()
        wq_cp(0, 0, 0).start()
        x_cp(1, 0, 0).start()
        wq_cp(1, 0, 0).start()
        if not peel:
            k_cp(0, 0, 0, 0).start()
            k_cp(1, 0, 0, 0).start()
        for bb in range(B):
            acc_ref[bb] = jnp.zeros((SQ, 2 * D), jnp.float32)
        if peel:
            wq_cp(0, 0, 0).wait()
            wq_cp(1, 0, 0).wait()
            k_cp(0, 0, 0, 0).start()
            k_cp(1, 0, 0, 0).start()
        v_cp(0, 0, 0, 0).start()
        v_cp(1, 0, 0, 0).start()
        wo_cp(0, 0, 0).start()
        wo_cp(1, 0, 0).start()

        lane = jax.lax.broadcasted_iota(jnp.int32, (SQ, 128), 1)

        def step(g, b, first):
            ws = g % 2
            if True:
                slot = b % 2
                i1 = g * B + b + 1
                last = i1 >= HG * B
                g1 = jnp.where(last, g, i1 // B)
                b1 = jnp.where(last, b, i1 % B)
                if not first and spos == 0:
                    start_step(g1, b1, 1 - slot)

                tasks = []
                if True:
                    for j in range(hb // 2):
                        for s in range(2):
                            tasks.append((s, 2 * j))
                            tasks.append((s, 2 * j + 1))
                n = len(tasks)
                qp, S, P, RL, OT, ON = {}, {}, {}, {}, {}, {}
                waited = set()

                def need(name, s):
                    if (name, s) in waited:
                        return
                    waited.add((name, s))
                    if name == 'x':
                        x_cp(s, b, slot).wait()
                    elif name == 'k':
                        k_cp(s, g, b, slot).wait()
                    elif name == 'v':
                        v_cp(s, g, b, slot).wait()
                        if s == 1 and first:
                            start_step(g1, b1, 1 - slot)
                    elif name == 'wo' and s == 0:
                        wo_cp(0, g, ws).wait()
                        wo_cp(1, g, ws).wait()

                if not first:
                    for nm in 'xkv':
                        for s in range(2):
                            need(nm, s)

                def qproj(s):
                    need('x', s)
                    q = jnp.dot(x_buf[slot, s], wq_buf[ws, s], preferred_element_type=jnp.float32) * qscale
                    q = q.astype(jnp.bfloat16)
                    for j in range(hb // 2):
                        q0 = q[:, 384 * j:384 * j + 128]
                        q1 = q[:, 384 * j + 128:384 * j + 256]
                        q2 = q[:, 384 * j + 256:384 * j + 384]
                        zero = jnp.zeros_like(q1)
                        qp[(s, 2 * j)] = jnp.concatenate([q0, jnp.where(lane < 64, q1, zero)], axis=1)
                        qp[(s, 2 * j + 1)] = jnp.concatenate([jnp.where(lane >= 64, q1, zero), q2], axis=1)

                def qk(t):
                    s, h = tasks[t]
                    need('k', s)
                    r0 = 384 * (h // 2) + 128 * (h % 2)
                    S[t] = jnp.dot(qp.pop((s, h)), k_buf[slot, s, r0:r0 + 256, :],
                                   preferred_element_type=jnp.float32)

                def sm(t):
                    s_ = S.pop(t)
                    m = jnp.max(s_, axis=1, keepdims=True)
                    p = jnp.exp2(s_ - m)
                    l = jnp.sum(p, axis=1, keepdims=True)
                    P[t] = p.astype(jnp.bfloat16)
                    RL[t] = 1.0 / l

                def pv(t):
                    s, h = tasks[t]
                    need('v', s)
                    OT[t] = jax.lax.dot_general(v_buf[slot, s, h * DH:(h + 1) * DH, :], P.pop(t),
                                                (((1,), (1,)), ((), ())),
                                                preferred_element_type=jnp.float32)

                def tr(t):
                    o = jnp.concatenate([OT.pop(t - 1), OT.pop(t)], axis=0).T
                    lane3 = jax.lax.broadcasted_iota(jnp.int32, (SQ, 384), 1)
                    o = o * jnp.where(lane3 < 192, RL.pop(t - 1), RL.pop(t))
                    ON[t] = o.astype(jnp.bfloat16)

                def op_all(s):
                    ts = [t for t in range(1, n, 2) if tasks[t][0] == s]
                    if first:
                        need('wo', s)
                    o = jnp.concatenate([ON.pop(t) for t in ts], axis=1)
                    r = jnp.dot(o, wo_buf[ws, s], preferred_element_type=jnp.float32)
                    acc_ref[b, :, s * D:(s + 1) * D] += r

                qb = -1
                qproj(0)
                if qb < 0:
                    qproj(1)
                qk(0)
                for u in range(n + 1):
                    if u == qb:
                        qproj(1)
                    if not first and spos == u + 1:
                        start_step(g1, b1, 1 - slot)
                    if u + 1 < n:
                        qk(u + 1)
                    if u < n:
                        sm(u)
                    if u == oa:
                        op_all(0)
                    if 0 <= u - 1 < n:
                        pv(u - 1)
                        if (u - 1) % 2 == 1:
                            tr(u - 1)
                if oa > n:
                    op_all(0)
                op_all(1)

                @pl.when(g == HG - 1)
                def _():
                    o_buf[b] = acc_ref[b].astype(jnp.bfloat16)
                    o_cp(b).start()


        def g_body(g, _):
            ws = g % 2

            @pl.when(g >= peel)
            def _():
                wq_cp(0, g, ws).wait()
                wq_cp(1, g, ws).wait()
                wo_cp(0, g, ws).wait()
                wo_cp(1, g, ws).wait()

            @pl.when(g + 1 < HG)
            def _():
                wq_cp(0, g + 1, 1 - ws).start()
                wq_cp(1, g + 1, 1 - ws).start()
                wo_cp(0, g + 1, 1 - ws).start()
                wo_cp(1, g + 1, 1 - ws).start()

            def b_body(b, _):
                step(g, b, False)
                return 0
            jax.lax.fori_loop(jnp.where(g == 0, peel, 0), B, b_body, 0)
            return 0

        if peel:
            step(0, 0, True)
        jax.lax.fori_loop(0, HG, g_body, 0)
        x_cp(0, 0, 0).wait()
        x_cp(1, 0, 0).wait()
        k_cp(0, 0, 0, 0).wait()
        k_cp(1, 0, 0, 0).wait()
        v_cp(0, 0, 0, 0).wait()
        v_cp(1, 0, 0, 0).wait()
        for bb in range(B):
            o_cp(bb).wait()

    def fn(A_x, A_k, A_v, A_wq, A_wo, B_x, B_k, B_v, B_wq, B_wo):
        t = lambda a: jnp.swapaxes(a, 2, 3).reshape(B, H * DH, SK)
        anys = pl.BlockSpec(memory_space=pl.ANY)
        return pl.pallas_call(
            kern,
            in_specs=[anys] * 10,
            out_specs=anys,
            out_shape=jax.ShapeDtypeStruct((B, SQ, 2 * D), jnp.bfloat16),
            scratch_shapes=[
                pltpu.VMEM((B, SQ, 2 * D), jnp.float32),
                pltpu.VMEM((2, 2, SQ, D), jnp.bfloat16),
                pltpu.VMEM((2, 2, HD, SK), jnp.bfloat16),
                pltpu.VMEM((2, 2, HD, SK), jnp.bfloat16),
                pltpu.VMEM((2, 2, D, HD), jnp.bfloat16),
                pltpu.VMEM((2, 2, HD, D), jnp.bfloat16),
                pltpu.VMEM((B, SQ, 2 * D), jnp.bfloat16),
                pltpu.SemaphoreType.DMA((2, 6)),
                pltpu.SemaphoreType.DMA((2, 4)),
                pltpu.SemaphoreType.DMA((B,)),
            ],
            compiler_params=pltpu.CompilerParams(
                vmem_limit_bytes=vmem * 1024 * 1024, disable_bounds_checks=nb),
        )(A_x, t(A_k), t(A_v), A_wq, A_wo, B_x, t(B_k), t(B_v), B_wq, B_wo)
    return fn


@jax.jit
def pallas_concat_heads__gqa_block_cached__gqa_block_cached__near_ridge_kernel(
        A_x, A_k_cache, A_v_cache, A_wq, A_wo, B_x, B_k_cache, B_v_cache, B_wq, B_wo):
    return make()(A_x, A_k_cache, A_v_cache, A_wq, A_wo, B_x, B_k_cache, B_v_cache, B_wq, B_wo)
```
